```python
import os as _os
_os.environ.setdefault("JAX_PLATFORMS", "cpu")
import jax
import jax.numpy as jnp

def _softmax(x, axis=-1):
    return jax.nn.softmax(x, axis=axis)
def _gelu(x):
    return jax.nn.gelu(x, approximate=True)
def _silu(x):
    return jax.nn.silu(x)
def _sigmoid(x):
    return jax.nn.sigmoid(x)
def _layernorm(x, axis=-1, eps=1e-5):
    m = jnp.mean(x, axis=axis, keepdims=True)
    v = jnp.var(x, axis=axis, keepdims=True)
    return (x - m) / jnp.sqrt(v + eps)
def _scatter_add(tgt, idx, src, axis=0):
    return tgt.at[idx].add(src)
def _segment_sum(src, seg, n):
    return jax.ops.segment_sum(src, seg, n)
class _Rng:
    def __init__(self, key):
        self._k = key
    def _next(self):
        self._k, sub = jax.random.split(self._k)
        return sub
    def normal(self, shape):
        return jax.random.normal(self._next(), shape, dtype=jnp.bfloat16)
    def randint(self, lo, hi, shape):
        return jax.random.randint(self._next(), shape, lo, hi, dtype=jnp.int32)
    def uniform(self, shape, lo=0.0, hi=1.0):
        return jax.random.uniform(self._next(), shape, jnp.bfloat16, lo, hi)
    def permutation(self, n):
        return jax.random.permutation(self._next(), n)


kernel_name = 'standalone__linear_kernel_hedgehog__prompt'

def setup_inputs():
    _rng = _Rng(jax.random.key(int.from_bytes(__import__("os").urandom(4), "little")))
    _w = (lambda a: (lambda t: t.astype(jnp.bfloat16) if jnp.issubdtype(t.dtype, jnp.floating) else t)(jnp.asarray(a)))
    B, S, D, H = 1, 2048, 1024, 32
    Dh = D // H
    return {
        "x": _w((lambda *s: _rng.normal(s) * 0.4)(B, S, D)),
        "wqkv": _w((lambda *s: _rng.normal(s) * 0.4)(D, 3 * D)),
        "w_phi": _w((lambda *s: _rng.normal(s) * 0.4)(H, Dh, Dh) * (Dh ** -0.5)),
        "wo": _w((lambda *s: _rng.normal(s) * 0.05)(D, D)),
    }

def reference(x, wqkv, w_phi, wo):
    B, S, D = x.shape
    H = 32; Dh = D // H
    qkv = (lambda x, *d: x.transpose(*d))((x @ wqkv).reshape(B, S, 3, H, Dh), 2, 0, 3, 1, 4)
    q, k, v = qkv[0], qkv[1], qkv[2]
    pq = jnp.einsum("bhsd,hdf->bhsf", q, w_phi)
    pk = jnp.einsum("bhsd,hdf->bhsf", k, w_phi)
    phi_q = jnp.concatenate([_softmax(pq, axis=-1), _softmax(-pq, axis=-1)], axis=-1)
    phi_k = jnp.concatenate([_softmax(pk, axis=-1), _softmax(-pk, axis=-1)], axis=-1)
    kv = jnp.einsum("bhsf,bhsd->bhfd", phi_k, v)
    z  = jnp.einsum("bhsf->bhf", phi_k)
    num = jnp.einsum("bhqf,bhfd->bhqd", phi_q, kv)
    den = jnp.einsum("bhqf,bhf->bhq", phi_q, z)[..., None] + 1e-6
    o = num / den
    return (lambda x, *d: x.transpose(*d))(o, 0, 2, 1, 3).reshape(B, S, D) @ wo
```

```python
import functools

import jax
import jax.numpy as jnp
import jax.experimental.pallas as pl
import jax.experimental.pallas.tpu as pltpu

H = 32
DH = 32
G = 4
NG = H // G
TS = 512

_NT = (((1,), (1,)), ((), ()))
_TN = (((0,), (0,)), ((), ()))


def _phi(pT, ts):
    p3 = pT.reshape(H, DH, ts)
    mx = jnp.max(p3, axis=1, keepdims=True)
    mn = jnp.min(p3, axis=1, keepdims=True)
    ep = jnp.exp(p3 - mx)
    em = jnp.exp(mn - p3)
    sp = jnp.sum(ep, axis=1, keepdims=True)
    sm = jnp.sum(em, axis=1, keepdims=True)
    pp = ep / sp
    pm = em / sm
    return pp.reshape(H * DH, ts), pm.reshape(H * DH, ts)


def _kernel(x_ref, wqkv_ref, wphi_ref, wo_ref, out_ref,
            wpT_ref, kv_ref, z_ref, kva_ref, *, d_model, ts):
    D = d_model
    phase = pl.program_id(0)
    i = pl.program_id(1)

    @pl.when(jnp.logical_and(phase == 0, i == 0))
    def _prologue():
        row = jax.lax.broadcasted_iota(jnp.int32, (128, 128), 0)
        col = jax.lax.broadcasted_iota(jnp.int32, (128, 128), 1)
        same_head = (row // DH) == (col // DH)
        for g in range(NG):
            w = wphi_ref[g * 128:(g + 1) * 128, :].astype(jnp.float32)
            w4 = jnp.concatenate([w] * G, axis=1)
            bd = jnp.where(same_head, w4, 0.0)
            bdT = bd.T.astype(jnp.bfloat16)
            for t in range(2):
                wcols = wqkv_ref[:, t * D + g * 128: t * D + (g + 1) * 128]
                r = jax.lax.dot_general(bdT, wcols, _NT,
                                        preferred_element_type=jnp.float32)
                wpT_ref[t * D + g * 128: t * D + (g + 1) * 128, :] = r.astype(jnp.bfloat16)
        kv_ref[...] = jnp.zeros_like(kv_ref)
        z_ref[...] = jnp.zeros_like(z_ref)

    xt = x_ref[...]

    @pl.when(phase == 0)
    def _kv_phase():
        pkT = jax.lax.dot_general(wpT_ref[D:2 * D, :], xt, _NT,
                                  preferred_element_type=jnp.float32)
        v = jnp.dot(xt, wqkv_ref[:, 2 * D:3 * D],
                    preferred_element_type=jnp.float32).astype(jnp.bfloat16)
        pp, pm = _phi(pkT, ts)
        for g in range(NG):
            f = jnp.concatenate([pp[g * 128:(g + 1) * 128], pm[g * 128:(g + 1) * 128]], axis=0)
            zpart = f[:, 0:128]
            for c in range(1, ts // 128):
                zpart = zpart + f[:, c * 128:(c + 1) * 128]
            z_ref[g] += zpart
            kv_ref[g] += jnp.dot(f.astype(jnp.bfloat16), v[:, g * 128:(g + 1) * 128],
                                 preferred_element_type=jnp.float32)

    @pl.when(jnp.logical_and(phase == 1, i == 0))
    def _mid():
        row = jax.lax.broadcasted_iota(jnp.int32, (128, 256), 0)
        col = jax.lax.broadcasted_iota(jnp.int32, (128, 256), 1)
        same_head = (row // DH) == ((col % 128) // DH)
        row8 = jax.lax.broadcasted_iota(jnp.int32, (16, 256), 0)
        col8 = jax.lax.broadcasted_iota(jnp.int32, (16, 256), 1)
        zsel = row8 == ((col8 % 128) // DH)
        for g in range(NG):
            kvT = kv_ref[g].T
            kva_ref[g, 0:128, :] = jnp.where(same_head, kvT, 0.0).astype(jnp.bfloat16)
            zT = jnp.sum(z_ref[g].T, axis=0, keepdims=True)
            zb = jnp.broadcast_to(zT, (16, 256))
            kva_ref[g, 128:144, :] = jnp.where(zsel, zb, 0.0).astype(jnp.bfloat16)

    @pl.when(phase == 1)
    def _q_phase():
        pqT = jax.lax.dot_general(wpT_ref[0:D, :], xt, _NT,
                                  preferred_element_type=jnp.float32)
        pp, pm = _phi(pqT, ts)
        os = []
        for g in range(NG):
            f = jnp.concatenate([pp[g * 128:(g + 1) * 128], pm[g * 128:(g + 1) * 128]], axis=0)
            nd = jnp.dot(kva_ref[g], f.astype(jnp.bfloat16),
                         preferred_element_type=jnp.float32)
            num = nd[0:128].reshape(G, DH, ts)
            den = nd[128:128 + G].reshape(G, 1, ts) + 1e-6
            os.append((num / den).reshape(128, ts))
        oT = jnp.concatenate(os, axis=0).astype(jnp.bfloat16)
        out = jax.lax.dot_general(oT, wo_ref[...], _TN,
                                  preferred_element_type=jnp.float32)
        out_ref[...] = out.astype(out_ref.dtype)


@jax.jit
def pallas_standalone__linear_kernel_hedgehog__prompt_kernel(
    x: jax.Array,
    wqkv: jax.Array,
    w_phi: jax.Array,
    wo: jax.Array,
):
    B, S, D = x.shape
    assert B == 1 and D == H * DH and S % TS == 0
    x2 = x.reshape(S, D)
    wphi2 = w_phi.reshape(H * DH, DH)
    n_t = S // TS

    out = pl.pallas_call(
        functools.partial(_kernel, d_model=D, ts=TS),
        grid=(2, n_t),
        in_specs=[
            pl.BlockSpec((TS, D), lambda p, i: (i, 0)),
            pl.BlockSpec((D, 3 * D), lambda p, i: (0, 0)),
            pl.BlockSpec((H * DH, DH), lambda p, i: (0, 0)),
            pl.BlockSpec((D, D), lambda p, i: (0, 0)),
        ],
        out_specs=pl.BlockSpec((TS, D), lambda p, i: (p * i, 0)),
        out_shape=jax.ShapeDtypeStruct((S, D), x.dtype),
        scratch_shapes=[
            pltpu.VMEM((2 * D, D), jnp.bfloat16),
            pltpu.VMEM((NG, 256, 128), jnp.float32),
            pltpu.VMEM((NG, 256, 128), jnp.float32),
            pltpu.VMEM((NG, 144, 256), jnp.bfloat16),
        ],
        compiler_params=pltpu.CompilerParams(
            dimension_semantics=("arbitrary", "arbitrary"),
            vmem_limit_bytes=100 * 1024 * 1024,
        ),
    )(x2, wqkv, wphi2, wo)
    return out.reshape(B, S, D)
```

```python
import functools

import jax
import jax.numpy as jnp
import jax.experimental.pallas as pl
import jax.experimental.pallas.tpu as pltpu

H = 32
DH = 32
G = 4
NG = H // G
NP = H // 2
TS = 512
CHUNKS = ((1, 0, 256), (1, 256, 256), (1, 512, 512), (2, 0, 1024))
WIN = 2

_NT = (((1,), (1,)), ((), ()))
_TN = (((0,), (0,)), ((), ()))


def _phi(pT, ts):
    nh = pT.shape[0] // DH
    p3 = pT.reshape(nh, DH, ts)
    mx = jnp.max(p3, axis=1, keepdims=True)
    mn = jnp.min(p3, axis=1, keepdims=True)
    ep = jnp.exp(p3 - mx)
    em = jnp.exp(mn - p3)
    sp = jnp.sum(ep, axis=1, keepdims=True)
    sm = jnp.sum(em, axis=1, keepdims=True)
    pp = ep / sp
    pm = em / sm
    return pp.reshape(nh * DH, ts), pm.reshape(nh * DH, ts)


def _pair_features(pp, pm, p):
    a, b = 2 * p, 2 * p + 1
    return jnp.concatenate([pp[a * DH:(a + 1) * DH], pm[a * DH:(a + 1) * DH],
                            pp[b * DH:(b + 1) * DH], pm[b * DH:(b + 1) * DH]], axis=0)


def _kernel(x_hbm, wqkv_hbm, wphi_ref, wo_hbm, out_ref,
            x_buf, wq_buf, wk_buf, wv_buf, wo_buf, bd_ref, wT_ref,
            kv_ref, z_ref, kva_ref, zc_ref, sem_x, sem_c, sem_w, *, d_model, seq):
    D = d_model
    ts = TS
    n_c = len(CHUNKS)
    n_t = seq // ts
    step = pl.program_id(0)

    def x_copy(t):
        return pltpu.make_async_copy(x_hbm.at[pl.ds(t * ts, ts), :],
                                     x_buf.at[pl.ds(t * ts, ts), :], sem_x.at[t])

    def w_chunk_copy(c):
        m, c0, nc = CHUNKS[c]
        buf = wk_buf if m == 1 else wv_buf
        return pltpu.make_async_copy(wqkv_hbm.at[:, pl.ds(m * D + c0, nc)],
                                     buf.at[:, pl.ds(c0, nc)], sem_c.at[c])

    wq_copy = pltpu.make_async_copy(wqkv_hbm.at[:, pl.ds(0, D)], wq_buf, sem_w.at[0])
    wo_copy = pltpu.make_async_copy(wo_hbm, wo_buf, sem_w.at[1])

    def fold(w_buf, g0, g1, t):
        for g in range(g0, g1):
            r = jax.lax.dot_general(bd_ref[g], w_buf[:, g * 128:(g + 1) * 128], _NT,
                                    preferred_element_type=jnp.float32)
            wT_ref[t * D + g * 128: t * D + (g + 1) * 128, :] = r.astype(jnp.bfloat16)

    def kv_features(pkT, p0, first):
        pp, pm = _phi(pkT, ts)
        fs = []
        for j in range(pkT.shape[0] // 64):
            f = _pair_features(pp, pm, j)
            zpart = f[:, 0:128]
            for c in range(1, ts // 128):
                zpart = zpart + f[:, c * 128:(c + 1) * 128]
            if first:
                z_ref[p0 + j] = zpart
            else:
                z_ref[p0 + j] += zpart
            fs.append(f.astype(jnp.bfloat16))
        return fs

    def kv_accumulate(fs, vT, p0, first):
        for j, f in enumerate(fs):
            kvp = jax.lax.dot_general(vT[j * 64:(j + 1) * 64], f, _NT,
                                      preferred_element_type=jnp.float32)
            if first:
                kv_ref[p0 + j] = kvp
            else:
                kv_ref[p0 + j] += kvp

    @pl.when(step == 0)
    def _kv_first():
        x_copy(0).start()
        for c in range(WIN):
            w_chunk_copy(c).start()
        row = jax.lax.broadcasted_iota(jnp.int32, (128, 128), 0)
        col = jax.lax.broadcasted_iota(jnp.int32, (128, 128), 1)
        same_head = (row // DH) == (col // DH)
        for g in range(NG):
            w = wphi_ref[g * 128:(g + 1) * 128, :].astype(jnp.float32)
            w4 = jnp.concatenate([w] * G, axis=1)
            bd = jnp.where(same_head, w4, 0.0)
            bd_ref[g] = bd.T.astype(jnp.bfloat16)
        x_copy(0).wait()
        xt = x_buf[0:ts, :]
        feats = []
        for c, (m, c0, nc) in enumerate(CHUNKS):
            w_chunk_copy(c).wait()
            if c + WIN < n_c:
                w_chunk_copy(c + WIN).start()
            elif c + WIN == n_c:
                x_copy(1).start()
            rows = slice(m * D + c0, m * D + c0 + nc)
            if m == 1:
                fold(wk_buf, c0 // 128, (c0 + nc) // 128, 1)
                pk = jax.lax.dot_general(wT_ref[rows, :], xt, _NT,
                                         preferred_element_type=jnp.float32)
                feats += kv_features(pk, c0 // 64, True)
            else:
                wT_ref[rows, :] = wv_buf[:, c0:c0 + nc].T
                vT = jax.lax.dot_general(wT_ref[rows, :], xt, _NT,
                                         preferred_element_type=jnp.float32).astype(jnp.bfloat16)
                kv_accumulate(feats[c0 // 64:(c0 + nc) // 64], vT, c0 // 64, True)

    @pl.when(step == 1)
    def _starts():
        for t in range(2, n_t):
            x_copy(t).start()
        wq_copy.start()
        wo_copy.start()

    @pl.when(jnp.logical_and(step > 0, step < n_t))
    def _kv_phase():
        x_copy(step).wait()
        xt = x_buf[pl.ds(pl.multiple_of(step * ts, ts), ts), :]
        kvT = jax.lax.dot_general(wT_ref[D:3 * D, :], xt, _NT,
                                  preferred_element_type=jnp.float32)
        fs = kv_features(kvT[0:D], 0, False)
        kv_accumulate(fs, kvT[D:2 * D].astype(jnp.bfloat16), 0, False)

    @pl.when(step == n_t)
    def _mid():
        wq_copy.wait()
        wo_copy.wait()
        fold(wq_buf, 0, NG, 0)
        row = jax.lax.broadcasted_iota(jnp.int32, (64, 128), 0)
        col = jax.lax.broadcasted_iota(jnp.int32, (64, 128), 1)
        same_head = (row // DH) == (col // (2 * DH))
        for p in range(NP):
            kva_ref[p] = jnp.where(same_head, kv_ref[p], 0.0).astype(jnp.bfloat16)
            zs = jnp.sum(z_ref[p], axis=1, keepdims=True)
            zc_ref[p] = jnp.broadcast_to(zs, (128, 128))

    @pl.when(step >= n_t)
    def _q_phase():
        t = step - n_t
        xt = x_buf[pl.ds(pl.multiple_of(t * ts, ts), ts), :]
        pqT = jax.lax.dot_general(wT_ref[0:D, :], xt, _NT,
                                  preferred_element_type=jnp.float32)
        pp, pm = _phi(pqT, ts)
        os = []
        for p in range(NP):
            f = _pair_features(pp, pm, p)
            num = jnp.dot(kva_ref[p], f.astype(jnp.bfloat16),
                          preferred_element_type=jnp.float32)
            fz = f * jnp.concatenate([zc_ref[p]] * (ts // 128), axis=1)
            den = jnp.sum(fz.reshape(2, 2 * DH, ts), axis=1, keepdims=True) + 1e-6
            os.append((num.reshape(2, DH, ts) / den).reshape(64, ts))
        oT = jnp.concatenate(os, axis=0).astype(jnp.bfloat16)
        out = jax.lax.dot_general(oT, wo_buf[...], _TN,
                                  preferred_element_type=jnp.float32)
        out_ref[...] = out.astype(out_ref.dtype)


@jax.jit
def pallas_standalone__linear_kernel_hedgehog__prompt_kernel(
    x: jax.Array,
    wqkv: jax.Array,
    w_phi: jax.Array,
    wo: jax.Array,
):
    B, S, D = x.shape
    assert B == 1 and D == H * DH and S % TS == 0
    x2 = x.reshape(S, D)
    wphi2 = w_phi.reshape(H * DH, DH)
    n_t = S // TS
    assert n_t >= 2

    out = pl.pallas_call(
        functools.partial(_kernel, d_model=D, seq=S),
        grid=(2 * n_t,),
        in_specs=[
            pl.BlockSpec(memory_space=pl.ANY),
            pl.BlockSpec(memory_space=pl.ANY),
            pl.BlockSpec((H * DH, DH), lambda s: (0, 0)),
            pl.BlockSpec(memory_space=pl.ANY),
        ],
        out_specs=pl.BlockSpec((TS, D), lambda s: (jnp.maximum(s - n_t, 0), 0)),
        out_shape=jax.ShapeDtypeStruct((S, D), x.dtype),
        scratch_shapes=[
            pltpu.VMEM((S, D), jnp.bfloat16),
            pltpu.VMEM((D, D), jnp.bfloat16),
            pltpu.VMEM((D, D), jnp.bfloat16),
            pltpu.VMEM((D, D), jnp.bfloat16),
            pltpu.VMEM((D, D), jnp.bfloat16),
            pltpu.VMEM((NG, 128, 128), jnp.bfloat16),
            pltpu.VMEM((3 * D, D), jnp.bfloat16),
            pltpu.VMEM((NP, 64, 128), jnp.float32),
            pltpu.VMEM((NP, 128, 128), jnp.float32),
            pltpu.VMEM((NP, 64, 128), jnp.bfloat16),
            pltpu.VMEM((NP, 128, 128), jnp.float32),
            pltpu.SemaphoreType.DMA((n_t,)),
            pltpu.SemaphoreType.DMA((len(CHUNKS),)),
            pltpu.SemaphoreType.DMA((2,)),
        ],
        compiler_params=pltpu.CompilerParams(
            dimension_semantics=("arbitrary",),
            vmem_limit_bytes=100 * 1024 * 1024,
        ),
    )(x2, wqkv, wphi2, wo)
    return out.reshape(B, S, D)
```

```python
import functools

import jax
import jax.numpy as jnp
import jax.experimental.pallas as pl
import jax.experimental.pallas.tpu as pltpu

H = 32
DH = 32
G = 4
NG = H // G
NP = H // 2
TS = 512
CHUNKS = ((1, 0, 256), (1, 256, 256), (1, 512, 512), (2, 0, 1024))
WIN = 2
OC = 256

_NT = (((1,), (1,)), ((), ()))


def _phi(pT, ts):
    nh = pT.shape[0] // DH
    p3 = pT.reshape(nh, DH, ts)
    mx = jnp.max(p3, axis=1, keepdims=True)
    mn = jnp.min(p3, axis=1, keepdims=True)
    ep = jnp.exp(p3 - mx)
    em = jnp.exp(mn - p3)
    sp = jnp.sum(ep, axis=1, keepdims=True)
    sm = jnp.sum(em, axis=1, keepdims=True)
    pp = ep / sp
    pm = em / sm
    return pp.reshape(nh * DH, ts), pm.reshape(nh * DH, ts)


def _pair_features(pp, pm, p):
    a, b = 2 * p, 2 * p + 1
    return jnp.concatenate([pp[a * DH:(a + 1) * DH], pm[a * DH:(a + 1) * DH],
                            pp[b * DH:(b + 1) * DH], pm[b * DH:(b + 1) * DH]], axis=0)


def _kernel(x_hbm, wqkv_hbm, wphi_hbm, wo_hbm, out_hbm,
            wphi_ref, out_buf, x_buf, wq_buf, wk_buf, wv_buf, wo_buf, bd_ref, wT_ref,
            kv_ref, z_ref, kva_ref, zc_ref, sem_x, sem_c, sem_w, sem_o, *, d_model, seq):
    D = d_model
    ts = TS
    n_c = len(CHUNKS)
    n_t = seq // ts
    n_oc = D // OC
    step = pl.program_id(0)

    def x_copy(t):
        return pltpu.make_async_copy(x_hbm.at[pl.ds(t * ts, ts), :],
                                     x_buf.at[pl.ds(t * ts, ts), :], sem_x.at[t])

    def w_chunk_copy(c):
        m, c0, nc = CHUNKS[c]
        buf = wk_buf if m == 1 else wv_buf
        return pltpu.make_async_copy(wqkv_hbm.at[:, pl.ds(m * D + c0, nc)],
                                     buf.at[:, pl.ds(c0, nc)], sem_c.at[c])

    def out_copy(t, c):
        return pltpu.make_async_copy(out_buf.at[pl.ds(t * ts, ts), pl.ds(c * OC, OC)],
                                     out_hbm.at[pl.ds(t * ts, ts), pl.ds(c * OC, OC)],
                                     sem_o.at[t * n_oc + c])

    wq_copy = pltpu.make_async_copy(wqkv_hbm.at[:, pl.ds(0, D)], wq_buf, sem_w.at[0])
    wo_copy = pltpu.make_async_copy(wo_hbm, wo_buf, sem_w.at[1])
    wphi_copy = pltpu.make_async_copy(wphi_hbm, wphi_ref, sem_w.at[2])

    def fold(w_buf, g0, g1, t):
        for g in range(g0, g1):
            r = jax.lax.dot_general(bd_ref[g], w_buf[:, g * 128:(g + 1) * 128], _NT,
                                    preferred_element_type=jnp.float32)
            wT_ref[t * D + g * 128: t * D + (g + 1) * 128, :] = r.astype(jnp.bfloat16)

    def kv_features(pkT, p0, first):
        pp, pm = _phi(pkT, ts)
        fs = []
        for j in range(pkT.shape[0] // 64):
            f = _pair_features(pp, pm, j)
            zpart = f[:, 0:128]
            for c in range(1, ts // 128):
                zpart = zpart + f[:, c * 128:(c + 1) * 128]
            if first:
                z_ref[p0 + j] = zpart
            else:
                z_ref[p0 + j] += zpart
            fs.append(f.astype(jnp.bfloat16))
        return fs

    def kv_accumulate(fs, vT, p0, first):
        for j, f in enumerate(fs):
            kvp = jax.lax.dot_general(vT[j * 64:(j + 1) * 64], f, _NT,
                                      preferred_element_type=jnp.float32)
            if first:
                kv_ref[p0 + j] = kvp
            else:
                kv_ref[p0 + j] += kvp

    @pl.when(step == 0)
    def _kv_first():
        wphi_copy.start()
        w_chunk_copy(0).start()
        x_copy(0).start()
        for c in range(1, WIN):
            w_chunk_copy(c).start()
        wphi_copy.wait()
        row = jax.lax.broadcasted_iota(jnp.int32, (128, 128), 0)
        col = jax.lax.broadcasted_iota(jnp.int32, (128, 128), 1)
        same_head = (row // DH) == (col // DH)
        for g in range(NG):
            w = wphi_ref[g * 128:(g + 1) * 128, :].astype(jnp.float32)
            w4 = jnp.concatenate([w] * G, axis=1)
            bd = jnp.where(same_head, w4, 0.0)
            bd_ref[g] = bd.T.astype(jnp.bfloat16)
        xt = None
        feats = []
        for c, (m, c0, nc) in enumerate(CHUNKS):
            w_chunk_copy(c).wait()
            if c + WIN < n_c:
                w_chunk_copy(c + WIN).start()
            elif c + WIN == n_c:
                x_copy(1).start()
            rows = slice(m * D + c0, m * D + c0 + nc)
            if m == 1:
                fold(wk_buf, c0 // 128, (c0 + nc) // 128, 1)
            else:
                wT_ref[rows, :] = wv_buf[:, c0:c0 + nc].T
            if xt is None:
                x_copy(0).wait()
                xt = x_buf[0:ts, :]
            proj = jax.lax.dot_general(wT_ref[rows, :], xt, _NT,
                                       preferred_element_type=jnp.float32)
            if m == 1:
                feats += kv_features(proj, c0 // 64, True)
            else:
                kv_accumulate(feats[c0 // 64:(c0 + nc) // 64], proj.astype(jnp.bfloat16),
                              c0 // 64, True)

    @pl.when(step == 1)
    def _starts():
        for t in range(2, n_t):
            x_copy(t).start()
        wq_copy.start()
        wo_copy.start()

    @pl.when(jnp.logical_and(step > 0, step < n_t))
    def _kv_phase():
        x_copy(step).wait()
        xt = x_buf[pl.ds(pl.multiple_of(step * ts, ts), ts), :]
        kvT = jax.lax.dot_general(wT_ref[D:3 * D, :], xt, _NT,
                                  preferred_element_type=jnp.float32)
        fs = kv_features(kvT[0:D], 0, False)
        kv_accumulate(fs, kvT[D:2 * D].astype(jnp.bfloat16), 0, False)

    @pl.when(step == n_t)
    def _mid():
        wq_copy.wait()
        wo_copy.wait()
        fold(wq_buf, 0, NG, 0)
        row = jax.lax.broadcasted_iota(jnp.int32, (64, 128), 0)
        col = jax.lax.broadcasted_iota(jnp.int32, (64, 128), 1)
        same_head = (row // DH) == (col // (2 * DH))
        for p in range(NP):
            kva_ref[p] = jnp.where(same_head, kv_ref[p], 0.0).astype(jnp.bfloat16)
            zs = jnp.sum(z_ref[p], axis=1, keepdims=True)
            zc_ref[p] = jnp.broadcast_to(zs, (128, 128))

    @pl.when(step >= n_t)
    def _q_phase():
        t = step - n_t
        xt = x_buf[pl.ds(pl.multiple_of(t * ts, ts), ts), :]
        pqT = jax.lax.dot_general(wT_ref[0:D, :], xt, _NT,
                                  preferred_element_type=jnp.float32)
        pp, pm = _phi(pqT, ts)
        os = []
        for p in range(NP):
            f = _pair_features(pp, pm, p)
            num = jnp.dot(kva_ref[p], f.astype(jnp.bfloat16),
                          preferred_element_type=jnp.float32)
            fz = f * jnp.concatenate([zc_ref[p]] * (ts // 128), axis=1)
            den = jnp.sum(fz.reshape(2, 2 * DH, ts), axis=1, keepdims=True) + 1e-6
            os.append((num.reshape(2, DH, ts) / den).reshape(64, ts))
        o = jnp.concatenate(os, axis=0).astype(jnp.bfloat16).T
        r0 = pl.multiple_of(t * ts, ts)
        for c in range(n_oc):
            out = jnp.dot(o, wo_buf[:, c * OC:(c + 1) * OC],
                          preferred_element_type=jnp.float32)
            out_buf[pl.ds(r0, ts), c * OC:(c + 1) * OC] = out.astype(out_buf.dtype)
            out_copy(t, c).start()

    @pl.when(step == 2 * n_t - 1)
    def _drain():
        for t in range(n_t):
            for c in range(n_oc):
                out_copy(t, c).wait()


@jax.jit
def pallas_standalone__linear_kernel_hedgehog__prompt_kernel(
    x: jax.Array,
    wqkv: jax.Array,
    w_phi: jax.Array,
    wo: jax.Array,
):
    B, S, D = x.shape
    assert B == 1 and D == H * DH and S % TS == 0
    x2 = x.reshape(S, D)
    wphi2 = w_phi.reshape(H * DH, DH)
    n_t = S // TS
    assert n_t >= 2

    out = pl.pallas_call(
        functools.partial(_kernel, d_model=D, seq=S),
        grid=(2 * n_t,),
        in_specs=[
            pl.BlockSpec(memory_space=pl.ANY),
            pl.BlockSpec(memory_space=pl.ANY),
            pl.BlockSpec(memory_space=pl.ANY),
            pl.BlockSpec(memory_space=pl.ANY),
        ],
        out_specs=pl.BlockSpec(memory_space=pl.ANY),
        out_shape=jax.ShapeDtypeStruct((S, D), x.dtype),
        scratch_shapes=[
            pltpu.VMEM((H * DH, DH), jnp.bfloat16),
            pltpu.VMEM((S, D), x.dtype),
            pltpu.VMEM((S, D), jnp.bfloat16),
            pltpu.VMEM((D, D), jnp.bfloat16),
            pltpu.VMEM((D, D), jnp.bfloat16),
            pltpu.VMEM((D, D), jnp.bfloat16),
            pltpu.VMEM((D, D), jnp.bfloat16),
            pltpu.VMEM((NG, 128, 128), jnp.bfloat16),
            pltpu.VMEM((3 * D, D), jnp.bfloat16),
            pltpu.VMEM((NP, 64, 128), jnp.float32),
            pltpu.VMEM((NP, 128, 128), jnp.float32),
            pltpu.VMEM((NP, 64, 128), jnp.bfloat16),
            pltpu.VMEM((NP, 128, 128), jnp.float32),
            pltpu.SemaphoreType.DMA((n_t,)),
            pltpu.SemaphoreType.DMA((len(CHUNKS),)),
            pltpu.SemaphoreType.DMA((3,)),
            pltpu.SemaphoreType.DMA((n_t * (D // OC),)),
        ],
        compiler_params=pltpu.CompilerParams(
            dimension_semantics=("arbitrary",),
            vmem_limit_bytes=100 * 1024 * 1024,
        ),
    )(x2, wqkv, wphi2, wo)
    return out.reshape(B, S, D)
```
